```python
import jax
import jax.numpy as jnp

def _softmax(x, axis=-1):
    return jax.nn.softmax(x, axis=axis)

def _gelu(x):
    return jax.nn.gelu(x, approximate=True)

def _silu(x):
    return jax.nn.silu(x)

def _sigmoid(x):
    return jax.nn.sigmoid(x)

def _layernorm(x, axis=-1, eps=1e-05):
    m = jnp.mean(x, axis=axis, keepdims=True)
    v = jnp.var(x, axis=axis, keepdims=True)
    return (x - m) / jnp.sqrt(v + eps)

def _scatter_add(tgt, idx, src, axis=0):
    return tgt.at[idx].add(src)

def _segment_sum(src, seg, n):
    return jax.ops.segment_sum(src, seg, n)

class _Rng:

    def __init__(self, key):
        self._k = key

    def _next(self):
        self._k, sub = jax.random.split(self._k)
        return sub

    def normal(self, shape):
        return jax.random.normal(self._next(), shape, dtype=jnp.bfloat16)

    def randint(self, lo, hi, shape):
        return jax.random.randint(self._next(), shape, lo, hi, dtype=jnp.int32)

    def uniform(self, shape, lo=0.0, hi=1.0):
        return jax.random.uniform(self._next(), shape, jnp.bfloat16, lo, hi)

    def permutation(self, n):
        return jax.random.permutation(self._next(), n)
kernel_name = 'adaLN_cond__sliding_block_cached__dense_activation_mish__decode'

def setup_inputs():
    _rng = _Rng(jax.random.key(int.from_bytes(__import__("os").urandom(4), "little")))
    _w = lambda a: (lambda t: t.astype(jnp.bfloat16) if jnp.issubdtype(t.dtype, jnp.floating) else t)(jnp.asarray(a))

    def _A_setup():
        B, Sq, D = (1, 1, 640)
        Hq, Hkv, Sk, Dh = (32, 32, 32768, 192)
        assert Hq % Hkv == 0, (Hq, Hkv)
        return {'x': _w((lambda *s: _rng.normal(s) * 0.05)(B, Sq, D)), 'k_cache': _w((lambda *s: _rng.normal(s) * 0.05)(B, Hkv, Sk, Dh)), 'v_cache': _w((lambda *s: _rng.normal(s) * 0.05)(B, Hkv, Sk, Dh)), 'wq': _w((lambda *s: _rng.normal(s) * 0.05)(D, Hq * Dh) * D ** (-0.5)), 'wo': _w((lambda *s: _rng.normal(s) * 0.05)(Hq * Dh, D) * (Hq * Dh) ** (-0.5))}
    _A_in = _A_setup()

    def _B_setup():
        B, S, D, F = (1, 1, 640, 1536)
        return {'x': _w((lambda *s: _rng.normal(s) * 0.05)(B, S, D)), 'w1': _w((lambda *s: _rng.normal(s) * 0.05)(D, F) * D ** (-0.5)), 'b1': _w((lambda *s: _rng.normal(s) * 0.05)(F)), 'w2': _w((lambda *s: _rng.normal(s) * 0.05)(F, D) * F ** (-0.5))}
    _B_in = _B_setup()
    return {'A_x': _A_in['x'], 'A_k_cache': _A_in['k_cache'], 'A_v_cache': _A_in['v_cache'], 'A_wq': _A_in['wq'], 'A_wo': _A_in['wo'], 'B_x': _B_in['x'], 'B_w1': _B_in['w1'], 'B_b1': _B_in['b1'], 'B_w2': _B_in['w2'], 'c': _w((lambda *s: _rng.normal(s) * 0.05)(1, 640)), 'w_mod': _w((lambda *s: _rng.normal(s) * 0.05)(640, 6 * 640) * 640 ** (-0.5))}

def reference(A_x, A_k_cache, A_v_cache, A_wq, A_wo, B_x, B_w1, B_b1, B_w2, c, w_mod):

    def _A_ref(x, k_cache, v_cache, wq, wo):
        B, Sq, D = x.shape
        Hq, Dh = (32, 192)
        Hkv, Sk = (k_cache.shape[1], k_cache.shape[2])
        W = min(4096, max(256, Sk // 4))
        rep = Hq // Hkv
        q = (lambda x, *d: x.transpose(*d))((x @ wq).reshape(B, Sq, Hq, Dh), 0, 2, 1, 3)
        k = jnp.repeat(k_cache[:, :, Sk - W:, :], rep, axis=1)
        v = jnp.repeat(v_cache[:, :, Sk - W:, :], rep, axis=1)
        scores = jnp.einsum('bhqd,bhkd->bhqk', q, k) * Dh ** (-0.5)
        p = _softmax(scores, axis=-1)
        o = jnp.einsum('bhqk,bhkd->bhqd', p, v)
        return (lambda x, *d: x.transpose(*d))(o, 0, 2, 1, 3).reshape(B, Sq, Hq * Dh) @ wo

    def _B_ref(x, w1, b1, w2):
        h = jnp.einsum('bsd,df->bsf', x, w1) + b1
        sp = jnp.log1p(jnp.exp(-jnp.abs(h))) + jnp.where(h > 0, h, jnp.zeros_like(h))
        act = h * jnp.tanh(sp)
        return jnp.einsum('bsf,fd->bsd', act, w2)
    x = A_x
    mod = (_silu(c) @ w_mod).reshape(c.shape[0], 6, 1, -1)
    sa, ca, ga, sb, cb, gb = (mod[:, 0].copy(), mod[:, 1].copy(), mod[:, 2].copy(), mod[:, 3].copy(), mod[:, 4].copy(), mod[:, 5].copy())
    h = _layernorm(x, axis=-1) * (1 + ca) + sa
    x = x + ga * _A_ref(h, A_k_cache, A_v_cache, A_wq, A_wo)
    h = _layernorm(x, axis=-1) * (1 + cb) + sb
    x = x + gb * _B_ref(h, B_w1, B_b1, B_w2)
    return x
```

```python
import functools

import jax
import jax.numpy as jnp
from jax import lax
from jax.experimental import pallas as pl
from jax.experimental.pallas import tpu as pltpu

F32 = jnp.float32
BF16 = jnp.bfloat16


def _layernorm(x, eps=1e-5):
    m = jnp.mean(x, axis=-1, keepdims=True)
    d = x - m
    v = jnp.mean(d * d, axis=-1, keepdims=True)
    return d / jnp.sqrt(v + eps)


def make(nbuf=3, wq_chunks=4, wo_chunks=4, w1_chunks=2, w2_chunks=4, prio_v=0):
    HQ, DH = 32, 192
    G = 2
    GD = G * DH
    NG = HQ // G
    R = 8

    def kernel(x_hbm, k_hbm, v_hbm, wq_hbm, wo_hbm, w1_hbm, b1_hbm, w2_hbm, c_hbm, wm_hbm,
               o_ref,
               x_v, c_v, b1_v, wm_v, wq_v, wo_v, w1_v, w2_v, k_v, v_v, q_s, o_s,
               sem_small, sem_wm, sem_wq, sem_wo, sem_w1, sem_w2, sem_k, sem_v):
        D = x_v.shape[-1]
        SK = k_hbm.shape[-1]
        W = k_v.shape[-1]
        F = w1_v.shape[-1]

        cp_x = pltpu.make_async_copy(x_hbm, x_v, sem_small.at[0])
        cp_c = pltpu.make_async_copy(c_hbm, c_v, sem_small.at[1])
        cp_b1 = pltpu.make_async_copy(b1_hbm, b1_v, sem_small.at[2])
        cp_wm = pltpu.make_async_copy(wm_hbm, wm_v, sem_wm)
        nq = HQ * DH // wq_chunks
        cp_wq = [pltpu.make_async_copy(wq_hbm.at[:, pl.ds(i * nq, nq)], wq_v.at[:, pl.ds(i * nq, nq)], sem_wq.at[i])
                 for i in range(wq_chunks)]
        no = HQ * DH // wo_chunks
        cp_wo = [pltpu.make_async_copy(wo_hbm.at[pl.ds(i * no, no), :], wo_v.at[pl.ds(i * no, no), :], sem_wo.at[i])
                 for i in range(wo_chunks)]
        n1 = F // w1_chunks
        cp_w1 = [pltpu.make_async_copy(w1_hbm.at[:, pl.ds(i * n1, n1)], w1_v.at[:, pl.ds(i * n1, n1)], sem_w1.at[i])
                 for i in range(w1_chunks)]
        n2 = F // w2_chunks
        cp_w2 = [pltpu.make_async_copy(w2_hbm.at[pl.ds(i * n2, n2), :], w2_v.at[pl.ds(i * n2, n2), :], sem_w2.at[i])
                 for i in range(w2_chunks)]

        def cp_k(g, slot):
            return pltpu.make_async_copy(
                k_hbm.at[pl.ds(pl.multiple_of(g * GD, GD), GD), pl.ds(SK - W, W)], k_v.at[slot], sem_k.at[slot])

        def cp_v(g, slot):
            return pltpu.make_async_copy(
                v_hbm.at[pl.ds(pl.multiple_of(g * GD, GD), GD), pl.ds(SK - W, W)], v_v.at[slot], sem_v.at[slot])

        cp_wm.start()
        cp_c.start()
        cp_x.start()
        cp_b1.start()
        for cp in cp_wq:
            cp.start()

        cp_c.wait()
        c = c_v[...].astype(F32)
        sc = jnp.broadcast_to(c * jax.nn.sigmoid(c), (R, D)).astype(BF16)
        cp_x.wait()
        x0 = jnp.broadcast_to(x_v[0].astype(F32), (R, D))
        ln0 = _layernorm(x0)
        cp_wm.wait()
        cp_k(0, 0).start()
        cp_v(0, 0).start(priority=prio_v)
        mod = jnp.dot(sc, wm_v[...], preferred_element_type=F32)
        sa, ca, ga, sb, cb, gb = [mod[:, i * D:(i + 1) * D] for i in range(6)]
        h = (ln0 * (1.0 + ca) + sa).astype(BF16)

        row = lax.broadcasted_iota(jnp.int32, (R, GD), 0)
        col = lax.broadcasted_iota(jnp.int32, (R, GD), 1)
        diag = (col >= row * DH) & (col < (row + 1) * DH)

        gpc = NG // wq_chunks
        for i in range(wq_chunks):
            cp_wq[i].wait()
            if i + 1 < nbuf - 1:
                cp_k(i + 1, i + 1).start()
                cp_v(i + 1, i + 1).start(priority=prio_v)
            q = jnp.dot(h, wq_v[:, i * nq:(i + 1) * nq], preferred_element_type=F32)
            for j in range(gpc):
                q_s[i * gpc + j] = jnp.where(diag, q[:, j * GD:(j + 1) * GD], 0.0)
        assert wq_chunks >= nbuf - 2

        ahead = nbuf - 1
        tail = cp_wo + cp_w1 + cp_w2
        per = -(-len(cp_wo) // (2 * ahead))

        def body(g, carry):
            slot = g % nbuf
            nxt = (g + ahead) % nbuf
            cp_k(g, slot).wait()

            @pl.when(g + ahead < NG)
            def _():
                cp_k(g + ahead, nxt).start()

            for t in range(ahead):
                @pl.when(g + ahead == NG + t)
                def _():
                    for cp in cp_wo[(2 * t) * per:(2 * t + 1) * per]:
                        cp.start()

            s = jnp.dot(q_s[g].astype(BF16), k_v[slot], preferred_element_type=F32) * (DH ** -0.5)
            m = jnp.max(s, axis=-1, keepdims=True)
            e = jnp.exp(s - m)
            l = jnp.sum(e, axis=-1, keepdims=True)
            cp_v(g, slot).wait()

            @pl.when(g + ahead < NG)
            def _():
                cp_v(g + ahead, nxt).start(priority=prio_v)

            for t in range(ahead):
                @pl.when(g + ahead == NG + t)
                def _():
                    for cp in cp_wo[(2 * t + 1) * per:(2 * t + 2) * per]:
                        cp.start()

            o = lax.dot_general(e.astype(BF16), v_v[slot], (((1,), (1,)), ((), ())), preferred_element_type=F32)
            o_s[g] = jnp.where(diag, o / l, 0.0)
            return carry

        lax.fori_loop(0, NG, body, 0)

        for cp in cp_w1:
            cp.start()
        gpo = NG // wo_chunks
        acc = jnp.zeros((R, D), F32)
        for i in range(wo_chunks):
            cp_wo[i].wait()
            if i < w2_chunks:
                cp_w2[i].start()
            oc = jnp.concatenate([o_s[i * gpo + j] for j in range(gpo)], axis=1).astype(BF16)
            acc = acc + jnp.dot(oc, wo_v[i * no:(i + 1) * no, :], preferred_element_type=F32)
        for i in range(wo_chunks, w2_chunks):
            cp_w2[i].start()
        attn = jnp.sum(acc, axis=0, keepdims=True)
        x1 = x0 + ga * attn
        h2 = (_layernorm(x1) * (1.0 + cb) + sb).astype(BF16)

        cp_b1.wait()
        b1 = b1_v[...].astype(F32).reshape(1, F)
        acts = []
        for i in range(w1_chunks):
            cp_w1[i].wait()
            u = jnp.dot(h2, w1_v[:, i * n1:(i + 1) * n1], preferred_element_type=F32) + b1[:, i * n1:(i + 1) * n1]
            sp = jnp.log1p(jnp.exp(-jnp.abs(u))) + jnp.where(u > 0, u, 0.0)
            acts.append((u * jnp.tanh(sp)).astype(BF16))
        act = jnp.concatenate(acts, axis=1)
        y = jnp.zeros((R, D), F32)
        for i in range(w2_chunks):
            cp_w2[i].wait()
            y = y + jnp.dot(act[:, i * n2:(i + 1) * n2], w2_v[i * n2:(i + 1) * n2, :], preferred_element_type=F32)
        out = x1 + gb * y
        o_ref[0] = out[0:1].astype(o_ref.dtype)

    def fn(A_x, A_k_cache, A_v_cache, A_wq, A_wo, B_x, B_w1, B_b1, B_w2, c, w_mod):
        del B_x
        _, Hkv, SK, _ = A_k_cache.shape
        W = min(4096, max(256, SK // 4))
        kt = jnp.swapaxes(A_k_cache, 2, 3).reshape(Hkv * DH, SK)
        vt = jnp.swapaxes(A_v_cache, 2, 3).reshape(Hkv * DH, SK)
        hbm = pl.BlockSpec(memory_space=pltpu.HBM)
        dma = pltpu.SemaphoreType.DMA
        return pl.pallas_call(
            kernel,
            out_shape=jax.ShapeDtypeStruct(A_x.shape, A_x.dtype),
            in_specs=[hbm] * 10,
            out_specs=pl.BlockSpec(memory_space=pltpu.VMEM),
            scratch_shapes=[
                pltpu.VMEM(A_x.shape, BF16), pltpu.VMEM(c.shape, BF16), pltpu.VMEM(B_b1.shape, BF16),
                pltpu.VMEM(w_mod.shape, BF16), pltpu.VMEM(A_wq.shape, BF16), pltpu.VMEM(A_wo.shape, BF16),
                pltpu.VMEM(B_w1.shape, BF16), pltpu.VMEM(B_w2.shape, BF16),
                pltpu.VMEM((nbuf, GD, W), BF16), pltpu.VMEM((nbuf, GD, W), BF16),
                pltpu.VMEM((NG, R, GD), F32), pltpu.VMEM((NG, R, GD), F32),
                dma((3,)), dma(()), dma((wq_chunks,)), dma((wo_chunks,)), dma((w1_chunks,)), dma((w2_chunks,)),
                dma((nbuf,)), dma((nbuf,)),
            ],
            compiler_params=pltpu.CompilerParams(vmem_limit_bytes=100 * 2**20),
        )(A_x, kt, vt, A_wq, A_wo, B_w1, B_b1, B_w2, c, w_mod)

    return fn


_impl = make()


@jax.jit
def pallas_adaLN_cond__sliding_block_cached__dense_activation_mish__decode_kernel(
    A_x, A_k_cache, A_v_cache, A_wq, A_wo, B_x, B_w1, B_b1, B_w2, c, w_mod):
    return _impl(A_x, A_k_cache, A_v_cache, A_wq, A_wo, B_x, B_w1, B_b1, B_w2, c, w_mod)
```

```python
import functools

import jax
import jax.numpy as jnp
from jax import lax
from jax.experimental import pallas as pl
from jax.experimental.pallas import tpu as pltpu

F32 = jnp.float32
BF16 = jnp.bfloat16


def _layernorm(x, eps=1e-5):
    m = jnp.mean(x, axis=-1, keepdims=True)
    d = x - m
    v = jnp.mean(d * d, axis=-1, keepdims=True)
    return d / jnp.sqrt(v + eps)


def _run(s0, s1, tasks):
    assert len(s0) == len(s1), (len(s0), len(s1))
    tasks = sorted(tasks, key=lambda t: t[0])
    ti = 0
    for i in range(len(s0)):
        while ti < len(tasks) and tasks[ti][0] <= i:
            tasks[ti][1]()
            ti += 1
        if s0[i] is not None:
            pltpu.make_async_copy(*s0[i]).start(priority=0)
        if s1[i] is not None:
            pltpu.make_async_copy(*s1[i]).start(priority=1)
    while ti < len(tasks):
        tasks[ti][1]()
        ti += 1


def _wait(buf, sem):
    pltpu.make_async_copy(buf, buf, sem).wait()


def make(kv_rows=192, piece=512, lag=12, w_rows=160, wo_rows=32, w2_rows=24, w2_tail=(6, 3), nobounds=False,
         pv_piece=512, ab=(), order=('wo', 'wm', 'w1', 'gb'), nslot=4):
    HQ, DH = 32, 192
    G = 2
    GD = G * DH
    NG = HQ // G
    R = 8

    def kernel(x_hbm, k_hbm, v_hbm, wq_hbm, wo_hbm, w1_hbm, b1_hbm, w2_hbm, c_hbm, wm_hbm,
               o_ref,
               x_v, c_v, b1_v, wm_v, wq_v, wo_v, w1_v, w2_v, k_v, v_v, q_s, o_s,
               sem_small, sem_wm, sem_wq, sem_wo, sem_w1, sem_w2, sem_k, sem_v):
        D = x_v.shape[-1]
        SK = k_hbm.shape[-1]
        W = k_v.shape[-1]
        F = w1_v.shape[-1]

        def col_tiles(src, dst, c0, c1, sem):
            return [(src.at[pl.ds(r, w_rows), pl.ds(c, 128)], dst.at[pl.ds(r, w_rows), pl.ds(c, 128)], sem)
                    for c in range(c0, c1, 128) for r in range(0, D, w_rows)]

        def row_tiles(src, dst, r0, r1, sem, rows):
            return [(src.at[pl.ds(r, rows), :], dst.at[pl.ds(r, rows), :], sem) for r in range(r0, r1, rows)]

        def head_tiles(src, dst, g, half, sem):
            slot = g % nslot
            base = g * GD + half * DH
            if not isinstance(g, int):
                base = pl.multiple_of(base, DH)
            return [(src.at[pl.ds(base + r, kv_rows), pl.ds(SK - W + c, 128)],
                     dst.at[slot, pl.ds(half * DH + r, kv_rows), pl.ds(c, 128)], sem.at[slot])
                    for c in range(0, W, 128) for r in range(0, DH, kv_rows)]

        def kt(g, half):
            return head_tiles(k_hbm, k_v, g, half, sem_k)

        def vt(g, half):
            return head_tiles(v_hbm, v_v, g, half, sem_v)

        row = lax.broadcasted_iota(jnp.int32, (R, GD), 0)
        col = lax.broadcasted_iota(jnp.int32, (R, GD), 1)
        diag = (col >= row * DH) & (col < (row + 1) * DH)

        st = {}
        nh = (W // 128) * (DH // kv_rows)
        ADV = F // w2_rows
        assert ADV % nh == 0 and ADV // nh in (1, 2)
        two = ADV // nh == 2

        head = col_tiles(wm_hbm, wm_v, 0, 2 * D, sem_wm.at[0])
        p_wm = len(head) // 2
        p_wq = []
        for g in range(NG):
            head += col_tiles(wq_hbm, wq_v, g * GD, (g + 1) * GD, sem_wq.at[g])
            p_wq.append(len(head) // 2)
        s0 = head[0::2] + kt(0, 0) + vt(0, 0)
        s1 = head[1::2] + kt(0, 1) + vt(0, 1) + kt(1, 1) + (vt(1, 1) if two else [])

        def t_small():
            _wait(c_v, sem_small.at[0])
            c = c_v[...].astype(F32)
            st['sc'] = jnp.broadcast_to(c * jax.nn.sigmoid(c), (R, D)).astype(BF16)
            _wait(x_v, sem_small.at[1])
            st['x0'] = jnp.broadcast_to(x_v[0].astype(F32), (R, D))
            st['ln0'] = _layernorm(st['x0'])

        def t_h():
            _wait(wm_v.at[:, pl.ds(0, 2 * D)], sem_wm.at[0])
            mod = jnp.zeros((R, 2 * D), F32) if 'now' in ab else jnp.dot(st['sc'], wm_v[:, 0:2 * D], preferred_element_type=F32)
            st['h'] = (st['ln0'] * (1.0 + mod[:, D:2 * D]) + mod[:, 0:D]).astype(BF16)

        def t_q(g):
            _wait(wq_v.at[:, pl.ds(g * GD, GD)], sem_wq.at[g])
            if 'now' in ab:
                return
            q = jnp.dot(st['h'], wq_v[:, g * GD:(g + 1) * GD], preferred_element_type=F32)
            q_s[g] = jnp.where(diag, q, 0.0)

        for cp in s1[:ADV]:
            pltpu.make_async_copy(*cp).start(priority=1)
        pltpu.make_async_copy(c_hbm, c_v, sem_small.at[0]).start()
        pltpu.make_async_copy(x_hbm, x_v, sem_small.at[1]).start()
        pltpu.make_async_copy(b1_hbm, b1_v, sem_small.at[2]).start()
        tasks = [(lag, t_small), (p_wm + lag, t_h)]
        tasks += [(p_wq[g] + lag, functools.partial(t_q, g)) for g in range(NG)]
        _run(s0, s1[ADV:], tasks)

        def attend(g, a0, a1, b0, b1):
            slot = g % nslot
            n = W // piece
            ss = []
            qg = q_s[g].astype(BF16)

            def t_qk(j):
                if 'noqk' in ab:
                    ss.append(jnp.zeros((R, piece), F32))
                    return
                ss.append(jnp.dot(qg, k_v[slot, :, j * piece:(j + 1) * piece], preferred_element_type=F32))

            _wait(k_v.at[slot], sem_k.at[slot])
            _run(a0, a1, [(j * len(a0) // n, functools.partial(t_qk, j)) for j in range(n)])
            s = jnp.concatenate(ss, axis=1) * (DH ** -0.5)
            m = jnp.max(s, axis=-1, keepdims=True)
            e = jnp.exp(s - m)
            l = jnp.sum(e, axis=-1, keepdims=True)
            p = e.astype(BF16)
            acc = []
            n2 = W // pv_piece

            def t_pv(j):
                if 'nopv' in ab:
                    acc.append(jnp.zeros((R, GD), F32))
                    return
                acc.append(lax.dot_general(p[:, j * pv_piece:(j + 1) * pv_piece],
                                           v_v[slot, :, j * pv_piece:(j + 1) * pv_piece],
                                           (((1,), (1,)), ((), ())), preferred_element_type=F32))

            _wait(v_v.at[slot], sem_v.at[slot])
            _run(b0, b1, [(1 + j * (len(b0) - 1) // n2, functools.partial(t_pv, j)) for j in range(n2)])
            o = functools.reduce(lambda a, b: a + b, acc)
            o_s[g] = jnp.where(diag, o / l, 0.0)

        def body(g, carry):
            if two:
                attend(g, kt(g + 1, 0), kt(g + 2, 1), vt(g + 1, 0), vt(g + 2, 1))
            else:
                attend(g, kt(g + 1, 0), vt(g + 1, 1), vt(g + 1, 0), kt(g + 2, 1))
            return carry

        lax.fori_loop(0, NG - 2, body, 0)

        tail = []
        n1 = 3
        f1 = F // n1
        p_wo, p_w1 = [], []
        for what in order:
            if what == 'wo':
                for g in range(NG):
                    tail += row_tiles(wo_hbm, wo_v, g * GD, (g + 1) * GD, sem_wo.at[g], wo_rows)
                    p_wo.append(len(tail) // 2)
            elif what == 'wm':
                tail += col_tiles(wm_hbm, wm_v, 2 * D, 5 * D, sem_wm.at[1])
                p_wm = len(tail) // 2
            elif what == 'w1':
                for i in range(n1):
                    tail += col_tiles(w1_hbm, w1_v, i * f1, (i + 1) * f1, sem_w1.at[i])
                    p_w1.append(len(tail) // 2)
            elif what == 'gb':
                tail += col_tiles(wm_hbm, wm_v, 5 * D, 6 * D, sem_wm.at[2])
                p_gb = len(tail) // 2
        edges = [0]
        for nt in (F // 128 - sum(w2_tail),) + tuple(w2_tail):
            edges.append(edges[-1] + nt * 128)
        last = []
        for i in range(len(edges) - 1):
            last += row_tiles(w2_hbm, w2_v, edges[i], edges[i + 1], sem_w2.at[i], w2_rows)
        g = NG - 1
        s0 = kt(g, 0) + vt(g, 0) + tail[0::2]
        s1 = ([] if two else vt(g, 1)) + tail[1::2] + last
        attend(NG - 2, s0[:nh], s1[:nh], s0[nh:2 * nh], s1[nh:2 * nh])
        attend(NG - 1, s0[2 * nh:3 * nh], s1[2 * nh:3 * nh], s0[3 * nh:4 * nh], s1[3 * nh:4 * nh])
        s0, s1 = s0[4 * nh:], s1[4 * nh:]
        off = lag - 2 * nh

        st['acc'] = jnp.zeros((R, D), F32)

        def t_wo(g):
            _wait(wo_v.at[pl.ds(g * GD, GD), :], sem_wo.at[g])
            if 'now' in ab:
                return
            st['acc'] = st['acc'] + jnp.dot(o_s[g].astype(BF16), wo_v[g * GD:(g + 1) * GD, :],
                                            preferred_element_type=F32)

        def t_mod():
            _wait(wm_v.at[:, pl.ds(2 * D, 3 * D)], sem_wm.at[1])
            st['mod'] = jnp.zeros((R, 3 * D), F32) if 'now' in ab else jnp.dot(st['sc'], wm_v[:, 2 * D:5 * D], preferred_element_type=F32)

        def t_h2():
            mod = st['mod']
            attn = jnp.sum(st['acc'], axis=0, keepdims=True)
            st['x1'] = st['x0'] + mod[:, 0:D] * attn
            st['h2'] = (_layernorm(st['x1']) * (1.0 + mod[:, 2 * D:3 * D]) + mod[:, D:2 * D]).astype(BF16)
            _wait(b1_v, sem_small.at[2])
            st['b1'] = b1_v[...].astype(F32).reshape(1, F)

        acts = []

        def t_w1(i):
            _wait(w1_v.at[:, pl.ds(i * f1, f1)], sem_w1.at[i])
            if 'now' in ab:
                acts.append(jnp.zeros((R, f1), BF16))
                return
            u = jnp.dot(st['h2'], w1_v[:, i * f1:(i + 1) * f1], preferred_element_type=F32)
            u = u + st['b1'][:, i * f1:(i + 1) * f1]
            sp = jnp.log1p(jnp.exp(-jnp.abs(u))) + jnp.where(u > 0, u, 0.0)
            acts.append((u * jnp.tanh(sp)).astype(BF16))

        def t_gb():
            _wait(wm_v.at[:, pl.ds(5 * D, D)], sem_wm.at[2])
            st['gb'] = jnp.zeros((R, D), F32) if 'now' in ab else jnp.dot(st['sc'], wm_v[:, 5 * D:6 * D], preferred_element_type=F32)

        tasks = [(max(p_wo[g] + off, g), functools.partial(t_wo, g)) for g in range(NG)]
        tasks += [(p_wm + off, t_mod)]
        p_h2 = max(t[0] for t in tasks) + 1
        tasks += [(p_h2, t_h2)]
        tasks += [(max(p_h2 + 1 + i, p_w1[i] + off), functools.partial(t_w1, i)) for i in range(n1)]
        tasks += [(p_gb + off, t_gb)]
        _run(s0, s1, tasks)
        act = jnp.concatenate(acts, axis=1)
        y = jnp.zeros((R, D), F32)
        for i in range(len(edges) - 1):
            a, b = edges[i], edges[i + 1]
            _wait(w2_v.at[pl.ds(a, b - a), :], sem_w2.at[i])
            if 'now' not in ab:
                y = y + jnp.dot(act[:, a:b], w2_v[a:b, :], preferred_element_type=F32)
        out = st['x1'] + st['gb'] * y
        o_ref[0] = out[0:1].astype(o_ref.dtype)

    def fn(A_x, A_k_cache, A_v_cache, A_wq, A_wo, B_x, B_w1, B_b1, B_w2, c, w_mod):
        del B_x
        _, Hkv, SK, _ = A_k_cache.shape
        W = min(4096, max(256, SK // 4))
        kt = jnp.swapaxes(A_k_cache, 2, 3).reshape(Hkv * DH, SK)
        vt = jnp.swapaxes(A_v_cache, 2, 3).reshape(Hkv * DH, SK)
        hbm = pl.BlockSpec(memory_space=pltpu.HBM)
        dma = pltpu.SemaphoreType.DMA
        return pl.pallas_call(
            kernel,
            out_shape=jax.ShapeDtypeStruct(A_x.shape, A_x.dtype),
            in_specs=[hbm] * 10,
            out_specs=pl.BlockSpec(memory_space=pltpu.VMEM),
            scratch_shapes=[
                pltpu.VMEM(A_x.shape, BF16), pltpu.VMEM(c.shape, BF16), pltpu.VMEM(B_b1.shape, BF16),
                pltpu.VMEM(w_mod.shape, BF16), pltpu.VMEM(A_wq.shape, BF16), pltpu.VMEM(A_wo.shape, BF16),
                pltpu.VMEM(B_w1.shape, BF16), pltpu.VMEM(B_w2.shape, BF16),
                pltpu.VMEM((nslot, GD, W), BF16), pltpu.VMEM((nslot, GD, W), BF16),
                pltpu.VMEM((NG, R, GD), F32), pltpu.VMEM((NG, R, GD), F32),
                dma((3,)), dma((3,)), dma((NG,)), dma((NG,)), dma((3,)), dma((len(w2_tail) + 1,)),
                dma((nslot,)), dma((nslot,)),
            ],
            compiler_params=pltpu.CompilerParams(vmem_limit_bytes=100 * 2**20, disable_bounds_checks=nobounds),
        )(A_x, kt, vt, A_wq, A_wo, B_w1, B_b1, B_w2, c, w_mod)

    return fn


_impl = make()


@jax.jit
def pallas_adaLN_cond__sliding_block_cached__dense_activation_mish__decode_kernel(
    A_x, A_k_cache, A_v_cache, A_wq, A_wo, B_x, B_w1, B_b1, B_w2, c, w_mod):
    return _impl(A_x, A_k_cache, A_v_cache, A_wq, A_wo, B_x, B_w1, B_b1, B_w2, c, w_mod)
```

```python
import functools

import jax
import jax.numpy as jnp
from jax import lax
from jax.experimental import pallas as pl
from jax.experimental.pallas import tpu as pltpu

F32 = jnp.float32
BF16 = jnp.bfloat16


def _layernorm(x, eps=1e-5):
    m = jnp.mean(x, axis=-1, keepdims=True)
    d = x - m
    v = jnp.mean(d * d, axis=-1, keepdims=True)
    return d / jnp.sqrt(v + eps)


def _run(s0, s1, tasks, first=0):
    assert len(s0) == len(s1), (len(s0), len(s1))
    tasks = sorted(tasks, key=lambda t: t[0])
    ti = 0
    for i in range(len(s0)):
        while ti < len(tasks) and tasks[ti][0] <= i:
            tasks[ti][1]()
            ti += 1
        for q in ((0, 1) if first == 0 else (1, 0)):
            pltpu.make_async_copy(*(s0, s1)[q][i]).start(priority=q)
    while ti < len(tasks):
        tasks[ti][1]()
        ti += 1


def _wait(buf, sem):
    pltpu.make_async_copy(buf, buf, sem).wait()


def make(kv_rows=192, piece=512, lag=14, w2_rows=24, w2_tail=(6, 3), nobounds=False, nosem=False, ab=(),
         wm_cfg=(2, 2, 8, 1280), wq_cfg=(5, 5, 8, 512), wo_cfg=(6, 3, 8, 640), w1_cfg=(1, 1, 16, 1536),
         wo_groups=2, first=0, kvlag=16):
    HQ, DH = 32, 192
    G = 2
    GD = G * DH
    NG = HQ // G
    R = 8
    NSLOT = 4

    def kernel(x_hbm, k_hbm, v_hbm, wq_hbm, wo_hbm, w1_hbm, b1_hbm, w2_hbm, c_hbm, wm_hbm,
               o_ref,
               x_v, c_v, b1_v, wm_v, wq_v, wo_v, w1_v, w2_v, kv_v, q_s, o_s, sems):
        D = x_v.shape[-1]
        SK = k_hbm.shape[-1]
        W = kv_v.shape[-1]
        F = w1_v.shape[-1]

        def tiles(src, dst, cfg, sem, b0=0, b1=None):
            A, na, rows, cols = cfg
            b1 = dst.shape[1] if b1 is None else b1
            out = []
            for a in range(0, A, na):
                for b in range(b0, b1, rows):
                    for c in range(0, dst.shape[2], cols):
                        sl = (pl.ds(a, na), pl.ds(b, rows), pl.ds(c, cols))
                        out.append((src.at[sl], dst.at[sl], sem))
            return out[:len(out) // 2], out[len(out) // 2:]

        def kv_tiles(src, which, g):
            slot = g % NSLOT
            base = g * GD
            if not isinstance(g, int):
                base = pl.multiple_of(base, GD)
            return [(src.at[pl.ds(base + r, kv_rows), pl.ds(SK - W + c, 128)],
                     kv_v.at[slot, which, pl.ds(r, kv_rows), pl.ds(c, 128)], sems.at[slot])
                    for r in range(0, GD, kv_rows) for c in range(0, W, 128)]

        def kt(g):
            return kv_tiles(k_hbm, 0, g)

        def vt(g):
            return kv_tiles(v_hbm, 1, g)

        def matvec(lhs, w, c0, c1):
            A, B, _ = w.shape
            if B % 128 == 0:
                parts = [jnp.dot(lhs[:, a * B:(a + 1) * B], w[a, :, c0:c1], preferred_element_type=F32) for a in range(A)]
                return functools.reduce(lambda u, v: u + v, parts)
            return jnp.dot(lhs, w[:, :, c0:c1].reshape(A * B, c1 - c0), preferred_element_type=F32)

        row = lax.broadcasted_iota(jnp.int32, (R, GD), 0)
        col = lax.broadcasted_iota(jnp.int32, (R, GD), 1)
        diag = (col >= row * DH) & (col < (row + 1) * DH)

        st = {}
        ng = (W // 128) * (GD // kv_rows)
        ADV = F // w2_rows
        assert ADV <= ng
        S_A, S_B, S_C = sems.at[NSLOT], sems.at[NSLOT + 1], sems.at[NSLOT + 2]

        m0, m1 = tiles(wm_hbm, wm_v, wm_cfg, S_B)
        q0, q1 = tiles(wq_hbm, wq_v, wq_cfg, S_C)
        s0 = m0 + q0 + kt(0)
        s1 = m1 + q1 + vt(0) + vt(1)[:ADV]
        small = [(c_hbm, c_v, S_A), (x_hbm, x_v, S_A), (b1_hbm, b1_v, S_A)]

        def t_small():
            for cp in small:
                pltpu.make_async_copy(*cp).wait()
            c = c_v[...].astype(F32)
            st['sc'] = jnp.broadcast_to(c * jax.nn.sigmoid(c), (R, D)).astype(BF16)
            st['x0'] = jnp.broadcast_to(x_v[0].astype(F32), (R, D))
            st['ln0'] = _layernorm(st['x0'])

        mods = []

        def t_mod(i):
            if i == 0:
                _wait(wm_v, S_B)
            mods.append(jnp.zeros((R, D), F32) if 'now' in ab else matvec(st['sc'], wm_v, i * D, (i + 1) * D))
            if i == 1:
                st['h'] = (st['ln0'] * (1.0 + mods[1]) + mods[0]).astype(BF16)

        def t_q(g):
            if g == 0:
                _wait(wq_v, S_C)
            if 'now' in ab:
                return
            q_s[g] = jnp.where(diag, matvec(st['h'], wq_v, g * GD, (g + 1) * GD), 0.0)

        for cp in s1[:ADV]:
            pltpu.make_async_copy(*cp).start(priority=1)
        for cp in small:
            pltpu.make_async_copy(*cp).start()
        tasks = [(lag, t_small)]
        tasks += [(len(m0) + lag + 4 * i, functools.partial(t_mod, i)) for i in range(6)]
        tasks += [(len(m0) + len(q0) + lag + (ng - lag) * g // NG, functools.partial(t_q, g)) for g in range(NG)]
        _run(s0, s1[ADV:], tasks, first)

        def attend(g, a0, a1):
            slot = g % NSLOT
            n = W // piece
            loc = {'s': [], 'o': []}

            def t_qk(j):
                if j == 0:
                    _wait(kv_v.at[slot], sems.at[slot])
                    loc['q'] = q_s[g].astype(BF16)
                if 'noqk' in ab:
                    loc['s'].append(jnp.zeros((R, piece), F32))
                    return
                loc['s'].append(jnp.dot(loc['q'], kv_v[slot, 0, :, j * piece:(j + 1) * piece],
                                        preferred_element_type=F32))

            def t_pv(j):
                if j == 0:
                    s = jnp.concatenate(loc['s'], axis=1) * (DH ** -0.5)
                    m = jnp.max(s, axis=-1, keepdims=True)
                    e = jnp.exp(s - m)
                    loc['l'] = jnp.sum(e, axis=-1, keepdims=True)
                    loc['p'] = e.astype(BF16)
                if 'nopv' in ab:
                    loc['o'].append(jnp.zeros((R, GD), F32))
                    return
                loc['o'].append(lax.dot_general(loc['p'][:, j * piece:(j + 1) * piece],
                                                kv_v[slot, 1, :, j * piece:(j + 1) * piece],
                                                (((1,), (1,)), ((), ())), preferred_element_type=F32))

            span = len(a0) - kvlag
            tasks = [(kvlag + j * span // (2 * n), functools.partial(t_qk, j)) for j in range(n)]
            tasks += [(kvlag + (n + j) * span // (2 * n), functools.partial(t_pv, j)) for j in range(n)]
            _run(a0, a1, tasks, first)
            o = functools.reduce(lambda a, b: a + b, loc['o'])
            o_s[g] = jnp.where(diag, o / loc['l'], 0.0)

        def body(g, carry):
            attend(g, kt(g + 1), vt(g + 1)[ADV:] + vt(g + 2)[:ADV])
            return carry

        lax.fori_loop(0, NG - 2, body, 0)

        Bo = wo_v.shape[1]
        wo_sem = [S_A, S_B, S_C][:wo_groups]
        t0, t1, p_wo = [], [], []
        for i in range(wo_groups):
            u0, u1 = tiles(wo_hbm, wo_v, wo_cfg, wo_sem[i], i * Bo // wo_groups, (i + 1) * Bo // wo_groups)
            t0 += u0
            t1 += u1
            p_wo.append(len(t0))
        w1_sem = sems.at[(NG - 4) % NSLOT]
        u0, u1 = tiles(w1_hbm, w1_v, w1_cfg, w1_sem)
        t0 += u0
        t1 += u1
        edges = [0]
        for nt in (F // 128 - sum(w2_tail),) + tuple(w2_tail):
            edges.append(edges[-1] + nt * 128)
        w2_sem = [sems.at[(NG - 3 + i) % NSLOT] for i in range(len(edges) - 1)]
        assert len(w2_sem) <= 3
        last = []
        for i in range(len(edges) - 1):
            last += [(w2_hbm.at[pl.ds(r, w2_rows), :], w2_v.at[pl.ds(r, w2_rows), :], w2_sem[i])
                     for r in range(edges[i], edges[i + 1], w2_rows)]
        s0 = kt(NG - 1) + t0
        s1 = vt(NG - 1)[ADV:] + t1 + last
        attend(NG - 2, s0[:ng], s1[:ng])
        attend(NG - 1, s0[ng:2 * ng], s1[ng:2 * ng])
        assert len(s1) - len(last) >= 2 * ng - ng + kvlag
        s0, s1 = s0[2 * ng:], s1[2 * ng:]
        off = lag - ng

        st['acc'] = jnp.zeros((R, D), F32)
        Ao = wo_v.shape[0]
        pb = 256 if (Bo // wo_groups) % 256 == 0 else 128

        def t_wo(i, a, b):
            if a == 0 and b == i * Bo // wo_groups:
                _wait(wo_v.at[:, pl.ds(b, Bo // wo_groups), :], wo_sem[i])
                if i == 0:
                    st['o'] = jnp.concatenate([o_s[g] for g in range(NG)], axis=1).astype(BF16)
            if 'now' in ab:
                return
            st['acc'] = st['acc'] + jnp.dot(st['o'][:, a * Bo + b:a * Bo + b + pb], wo_v[a, b:b + pb, :],
                                            preferred_element_type=F32)

        tasks = []
        pos = 0
        for i in range(wo_groups):
            pos = max(pos, p_wo[i] + off)
            for a in range(Ao):
                for b in range(i * Bo // wo_groups, (i + 1) * Bo // wo_groups, pb):
                    tasks.append((pos, functools.partial(t_wo, i, a, b)))
                    pos += 1
        _run(s0, s1, tasks, first)

        sa, ca, ga, sb, cb, gb = mods
        attn = jnp.sum(st['acc'], axis=0, keepdims=True)
        x1 = st['x0'] + ga * attn
        h2 = (_layernorm(x1) * (1.0 + cb) + sb).astype(BF16)
        b1 = b1_v[...].astype(F32).reshape(1, F)
        _wait(w1_v, w1_sem)
        u = (jnp.zeros((R, F), F32) if 'now' in ab else matvec(h2, w1_v, 0, F)) + b1
        sp = jnp.log1p(jnp.exp(-jnp.abs(u))) + jnp.where(u > 0, u, 0.0)
        act = (u * jnp.tanh(sp)).astype(BF16)
        y = jnp.zeros((R, D), F32)
        for i in range(len(edges) - 1):
            a, b = edges[i], edges[i + 1]
            _wait(w2_v.at[pl.ds(a, b - a), :], w2_sem[i])
            if 'now' not in ab:
                y = y + jnp.dot(act[:, a:b], w2_v[a:b, :], preferred_element_type=F32)
        out = x1 + gb * y
        o_ref[0] = out[0:1].astype(o_ref.dtype)

    def fn(A_x, A_k_cache, A_v_cache, A_wq, A_wo, B_x, B_w1, B_b1, B_w2, c, w_mod):
        del B_x
        _, Hkv, SK, _ = A_k_cache.shape
        W = min(4096, max(256, SK // 4))
        kt = jnp.swapaxes(A_k_cache, 2, 3).reshape(Hkv * DH, SK)
        vt = jnp.swapaxes(A_v_cache, 2, 3).reshape(Hkv * DH, SK)

        def slabs(w, cfg):
            return w.reshape(cfg[0], w.shape[0] // cfg[0], w.shape[1])

        wm, wq, wo, w1 = slabs(w_mod, wm_cfg), slabs(A_wq, wq_cfg), slabs(A_wo, wo_cfg), slabs(B_w1, w1_cfg)
        hbm = pl.BlockSpec(memory_space=pltpu.HBM)
        return pl.pallas_call(
            kernel,
            out_shape=jax.ShapeDtypeStruct(A_x.shape, A_x.dtype),
            in_specs=[hbm] * 10,
            out_specs=pl.BlockSpec(memory_space=pltpu.VMEM),
            scratch_shapes=[
                pltpu.VMEM(A_x.shape, BF16), pltpu.VMEM(c.shape, BF16), pltpu.VMEM(B_b1.shape, BF16),
                pltpu.VMEM(wm.shape, BF16), pltpu.VMEM(wq.shape, BF16), pltpu.VMEM(wo.shape, BF16),
                pltpu.VMEM(w1.shape, BF16), pltpu.VMEM(B_w2.shape, BF16),
                pltpu.VMEM((NSLOT, 2, GD, W), BF16),
                pltpu.VMEM((NG, R, GD), F32), pltpu.VMEM((NG, R, GD), F32),
                pltpu.SemaphoreType.DMA((NSLOT + 3,)),
            ],
            compiler_params=pltpu.CompilerParams(vmem_limit_bytes=100 * 2**20, disable_bounds_checks=nobounds,
                                                 disable_semaphore_checks=nosem),
        )(A_x, kt, vt, wq, wo, w1, B_b1, B_w2, c, wm)

    return fn


_impl = make(kv_rows=96)


@jax.jit
def pallas_adaLN_cond__sliding_block_cached__dense_activation_mish__decode_kernel(
    A_x, A_k_cache, A_v_cache, A_wq, A_wo, B_x, B_w1, B_b1, B_w2, c, w_mod):
    return _impl(A_x, A_k_cache, A_v_cache, A_wq, A_wo, B_x, B_w1, B_b1, B_w2, c, w_mod)
```

```python
import functools

import jax
import jax.numpy as jnp
from jax import lax
import jax.experimental.pallas as pl
import jax.experimental.pallas.tpu as pltpu

F32 = jnp.float32
BF16 = jnp.bfloat16

LANES = 128
ROWS = 8
PAIR = 2
NSLOT = 4
KV_ROWS = 96
WM_COLS = 384
WQ_COLS = 384
WO_SLABS = 8
W1_COLS = 768
W2_ROWS = 24
W2_VPU = (288, 72, 24)
AHEAD = 24
LAG = 14
KV_LAG = 32


def _layernorm(x, eps=1e-5):
    d = x - jnp.mean(x, axis=-1, keepdims=True)
    return d / jnp.sqrt(jnp.mean(d * d, axis=-1, keepdims=True) + eps)


def _mish(u):
    softplus = jnp.log1p(jnp.exp(-jnp.abs(u))) + jnp.where(u > 0, u, 0.0)
    return u * jnp.tanh(softplus)


def _sum(parts):
    return functools.reduce(lambda a, b: a + b, parts)


def _halves(copies):
    assert len(copies) % 2 == 0
    return copies[:len(copies) // 2], copies[len(copies) // 2:]


def _stream(q0, q1, tasks):
    assert len(q0) == len(q1)
    tasks = sorted(tasks, key=lambda t: t[0])
    for step, copies in enumerate(zip(q0, q1)):
        while tasks and tasks[0][0] <= step:
            tasks.pop(0)[1]()
        for priority, (src, dst, sem) in enumerate(copies):
            pltpu.make_async_copy(src, dst, sem).start(priority=priority)
    for _, fn in tasks:
        fn()


def _wait_all(buf, sem):
    pltpu.make_async_copy(buf, buf, sem).wait()


def _aligned(i, n):
    return i if isinstance(i, int) else pl.multiple_of(i, n)


def _kernel(x_hbm, k_hbm, v_hbm, wq_hbm, wo_hbm, w1_hbm, b1_hbm, w2_hbm, c_hbm, wm_hbm, o_ref,
            x_v, c_v, b1_v, wa_v, wo_v, w1_v, w2_v, kv_v, sems, *, head_dim):
    D, F = w1_v.shape
    GD, W = kv_v.shape[2:]
    SK = k_hbm.shape[1]
    NG = k_hbm.shape[0] // GD
    NM, NQ = wm_hbm.shape[2], wq_hbm.shape[2]
    steps = (GD // KV_ROWS) * (W // LANES)
    assert NG >= NSLOT and AHEAD <= steps

    sem_small = sem_w1 = sems.at[NSLOT]
    sem_wm, sem_wq, sem_wo = sems.at[2], sems.at[3], sems.at[NSLOT + 1]
    sem_w2 = [sems.at[(NG - 4) % NSLOT], sems.at[(NG - 3) % NSLOT], sems.at[(NG - 2) % NSLOT], sems.at[NSLOT + 1]]

    def wa_copies(src, col0, cols, sem):
        return [(src.at[:, pl.ds(r, 8), pl.ds(c, cols)], wa_v.at[:, pl.ds(r, 8), pl.ds(col0 + c, cols)], sem)
                for r in range(0, src.shape[1], 8) for c in range(0, src.shape[2], cols)]

    def kv_copies(which, g):
        src, slot, base = (k_hbm, v_hbm)[which], g % NSLOT, _aligned(g * GD, GD)
        return [(src.at[pl.ds(base + r, KV_ROWS), pl.ds(SK - W + c, LANES)],
                 kv_v.at[slot, which, pl.ds(r, KV_ROWS), pl.ds(c, LANES)], sems.at[slot])
                for r in range(0, GD, KV_ROWS) for c in range(0, W, LANES)]

    def wa_matmul(lhs, col0, cols):
        return _sum([jnp.dot(lhs[:, a * LANES:(a + 1) * LANES], wa_v[a, :, pl.ds(col0, cols)],
                             preferred_element_type=F32) for a in range(wa_v.shape[0])])

    small = [(c_hbm, c_v, sem_small), (x_hbm, x_v, sem_small), (b1_hbm, b1_v, sem_small)]
    wm0, wm1 = _halves(wa_copies(wm_hbm, 0, WM_COLS, sem_wm))
    wq0, wq1 = _halves(wa_copies(wq_hbm, NM, WQ_COLS, sem_wq))
    na = wo_v.shape[0] // 2
    wo0, wo1 = _halves([(wo_hbm.at[pl.ds(a, na), pl.ds(r, 8), :], wo_v.at[pl.ds(a, na), pl.ds(r, 8), :], sem_wo)
                        for a in (0, na) for r in range(0, wo_v.shape[1], 8)])
    q0 = wm0 + wq0 + wo0 + kv_copies(0, 0)
    q1 = wm1 + wq1 + wo1 + kv_copies(1, 0) + kv_copies(1, 1)[:AHEAD]
    val, mod = {}, []

    def load_small():
        for copy in small:
            pltpu.make_async_copy(*copy).wait()
        c = c_v[...].astype(F32)
        val['silu_c'] = jnp.broadcast_to(c * jax.nn.sigmoid(c), (ROWS, D)).astype(BF16)
        val['x'] = jnp.broadcast_to(x_v[0].astype(F32), (ROWS, D))

    def modulation(i):
        if i == 0:
            _wait_all(wa_v.at[:, :, pl.ds(0, NM)], sem_wm)
        mod.append(wa_matmul(val['silu_c'], i * D, D))

    def wait_projections():
        _wait_all(wa_v.at[:, :, pl.ds(NM, NQ)], sem_wq)
        _wait_all(wo_v, sem_wo)

    for copy in q1[:AHEAD]:
        pltpu.make_async_copy(*copy).start(priority=1)
    for copy in small:
        pltpu.make_async_copy(*copy).start()
    _stream(q0, q1[AHEAD:],
            [(LAG, load_small)]
            + [(len(wm0) + LAG + 6 * i, functools.partial(modulation, i)) for i in range(NM // D)]
            + [(len(wm0) + len(wq0) + len(wo0) + LAG, wait_projections)])
    shift_a, scale_a, gate_a, shift_b, scale_b, gate_b = mod
    h = (_layernorm(val['x']) * (1.0 + scale_a) + shift_a).astype(BF16)

    head = lax.broadcasted_iota(jnp.int32, (ROWS, GD), 0)
    col = lax.broadcasted_iota(jnp.int32, (ROWS, GD), 1)
    own = (col >= head * head_dim) & (col < (head + 1) * head_dim)
    piece = 4 * LANES
    n = W // piece

    def attend(g, acc, q0, q1):
        slot = g % NSLOT
        loc = {'s': [], 'o': []}

        def scores(j):
            if j == 0:
                q = wa_matmul(h, _aligned(NM + g * GD, LANES), GD)
                loc['q'] = jnp.where(own, q, 0.0).astype(BF16)
                _wait_all(kv_v.at[slot], sems.at[slot])
            loc['s'].append(jnp.dot(loc['q'], kv_v[slot, 0, :, pl.ds(j * piece, piece)],
                                    preferred_element_type=F32))

        def mix(j):
            if j == 0:
                s = jnp.concatenate(loc['s'], axis=1) * head_dim ** -0.5
                e = jnp.exp(s - jnp.max(s, axis=-1, keepdims=True))
                loc['l'] = jnp.sum(e, axis=-1, keepdims=True)
                loc['p'] = e.astype(BF16)
            loc['o'].append(lax.dot_general(loc['p'][:, j * piece:(j + 1) * piece],
                                            kv_v[slot, 1, :, pl.ds(j * piece, piece)],
                                            (((1,), (1,)), ((), ())), preferred_element_type=F32))

        span = max(len(q0) - KV_LAG - 4, 0)
        _stream(q0, q1,
                [(KV_LAG + j * span // (2 * n), functools.partial(scores, j)) for j in range(n)]
                + [(KV_LAG + (n + j) * span // (2 * n), functools.partial(mix, j)) for j in range(n)])
        o = jnp.where(own, _sum(loc['o']) / loc['l'], 0.0).astype(BF16)
        per_slab = wo_v.shape[1] // GD
        wo_g = wo_v[g // per_slab, pl.ds(_aligned((g % per_slab) * GD, GD), GD), :]
        return acc + jnp.dot(o, wo_g, preferred_element_type=F32)

    acc = lax.fori_loop(
        0, NG - 2,
        lambda g, acc: attend(g, acc, kv_copies(0, g + 1),
                              kv_copies(1, g + 1)[AHEAD:] + kv_copies(1, g + 2)[:AHEAD]),
        jnp.zeros((ROWS, D), F32))

    w1_0, w1_1 = _halves([(w1_hbm.at[pl.ds(r, 8), pl.ds(c, W1_COLS)], w1_v.at[pl.ds(r, 8), pl.ds(c, W1_COLS)], sem_w1)
                          for r in range(0, D, 8) for c in range(0, F, W1_COLS)])
    edges = [0, F - sum(W2_VPU)]
    for rows in W2_VPU:
        edges.append(edges[-1] + rows)
    w2 = [(w2_hbm.at[pl.ds(r, W2_ROWS), :], w2_v.at[pl.ds(r, W2_ROWS), :], sem)
          for lo, hi, sem in zip(edges, edges[1:], sem_w2) for r in range(lo, hi, W2_ROWS)]
    shared = len(w2) - AHEAD
    q0 = kv_copies(0, NG - 1) + w1_0 + w2[0:shared:2]
    q1 = kv_copies(1, NG - 1)[AHEAD:] + w1_1 + w2[1:shared:2] + w2[shared:]
    assert not any(sem is sem_w2[2] for _, _, sem in q0[:steps] + q1[:steps])
    acc = attend(NG - 2, acc, q0[:steps], q1[:steps])
    acc = attend(NG - 1, acc, q0[steps:], q1[steps:])

    x1 = val['x'] + gate_a * jnp.sum(acc, axis=0, keepdims=True)
    h2 = (_layernorm(x1) * (1.0 + scale_b) + shift_b).astype(BF16)
    b1 = b1_v[...].astype(F32).reshape(1, F)
    _wait_all(w1_v, sem_w1)
    act = jnp.concatenate(
        [_mish(jnp.dot(h2, w1_v[:, c:c + piece], preferred_element_type=F32) + b1[:, c:c + piece]).astype(BF16)
         for c in range(0, F, piece)], axis=1)

    first = edges[1] // LANES * LANES
    act_col = jnp.concatenate(
        [jnp.broadcast_to(act[0:1, c:c + LANES].astype(F32), (LANES, LANES)).T for c in range(first, F, LANES)],
        axis=0)
    _wait_all(w2_v.at[pl.ds(0, edges[1]), :], sem_w2[0])
    y = jnp.dot(act[:, :edges[1]], w2_v[:edges[1], :], preferred_element_type=F32)
    out = (x1 + gate_b * y)[0:1]
    rest = []
    for lo, hi, sem in zip(edges[1:], edges[2:], sem_w2[1:]):
        _wait_all(w2_v.at[pl.ds(lo, hi - lo), :], sem)
        prod = w2_v[lo:hi, :].astype(F32) * jnp.concatenate([act_col[lo - first:hi - first]] * (D // LANES), axis=1)
        rest.append(jnp.sum(prod.reshape((hi - lo) // 8, 8, D), axis=0))
    out = out + gate_b[0:1] * jnp.sum(_sum(rest), axis=0, keepdims=True)
    o_ref[0] = out.astype(o_ref.dtype)


@jax.jit
def pallas_adaLN_cond__sliding_block_cached__dense_activation_mish__decode_kernel(
    A_x: jax.Array,
    A_k_cache: jax.Array,
    A_v_cache: jax.Array,
    A_wq: jax.Array,
    A_wo: jax.Array,
    B_x: jax.Array,
    B_w1: jax.Array,
    B_b1: jax.Array,
    B_w2: jax.Array,
    c: jax.Array,
    w_mod: jax.Array,
):
    del B_x
    batch, heads, seq, head_dim = A_k_cache.shape
    D, F = B_w1.shape
    window = min(4096, max(256, seq // 4))
    pair_rows = PAIR * head_dim
    assert A_x.shape == (1, 1, D) and batch == 1 and A_wq.shape == (D, heads * head_dim)
    assert w_mod.shape == (D, 6 * D) and D % LANES == 0 and pair_rows % LANES == 0 and pair_rows % KV_ROWS == 0
    assert window % (4 * LANES) == 0 and seq % LANES == 0 and (heads * head_dim) % (WO_SLABS * pair_rows) == 0
    assert (6 * D) % WM_COLS == 0 and (heads * head_dim) % WQ_COLS == 0
    assert F % W1_COLS == 0 and F % (4 * LANES) == 0 and (F - sum(W2_VPU)) % LANES == 0
    assert all(rows % W2_ROWS == 0 for rows in (F,) + W2_VPU)

    def seq_minor(cache):
        return jnp.swapaxes(cache, 2, 3).reshape(heads * head_dim, seq)

    def slabs(w, count):
        return w.reshape(count, w.shape[0] // count, w.shape[1])

    wo = slabs(A_wo, WO_SLABS)
    return pl.pallas_call(
        functools.partial(_kernel, head_dim=head_dim),
        out_shape=jax.ShapeDtypeStruct(A_x.shape, A_x.dtype),
        in_specs=[pl.BlockSpec(memory_space=pltpu.HBM)] * 10,
        out_specs=pl.BlockSpec(memory_space=pltpu.VMEM),
        scratch_shapes=[
            pltpu.VMEM(A_x.shape, A_x.dtype),
            pltpu.VMEM(c.shape, c.dtype),
            pltpu.VMEM(B_b1.shape, B_b1.dtype),
            pltpu.VMEM((D // LANES, LANES, 6 * D + heads * head_dim), A_wq.dtype),
            pltpu.VMEM(wo.shape, wo.dtype),
            pltpu.VMEM(B_w1.shape, B_w1.dtype),
            pltpu.VMEM(B_w2.shape, B_w2.dtype),
            pltpu.VMEM((NSLOT, 2, pair_rows, window), A_k_cache.dtype),
            pltpu.SemaphoreType.DMA((NSLOT + 2,)),
        ],
        compiler_params=pltpu.CompilerParams(
            vmem_limit_bytes=80 * 2**20, disable_bounds_checks=True, disable_semaphore_checks=True),
    )(A_x, seq_minor(A_k_cache), seq_minor(A_v_cache), slabs(A_wq, D // LANES), wo, B_w1, B_b1, B_w2, c,
      slabs(w_mod, D // LANES))
```
